```python
import os as _os
_os.environ.setdefault('JAX_PLATFORMS', 'cpu')
import jax
import jax.numpy as jnp

def _softmax(x, axis=-1):
    return jax.nn.softmax(x, axis=axis)

def _gelu(x):
    return jax.nn.gelu(x, approximate=True)

def _silu(x):
    return jax.nn.silu(x)

def _sigmoid(x):
    return jax.nn.sigmoid(x)

def _layernorm(x, axis=-1, eps=1e-05):
    m = jnp.mean(x, axis=axis, keepdims=True)
    v = jnp.var(x, axis=axis, keepdims=True)
    return (x - m) / jnp.sqrt(v + eps)

def _scatter_add(tgt, idx, src, axis=0):
    return tgt.at[idx].add(src)

def _segment_sum(src, seg, n):
    return jax.ops.segment_sum(src, seg, n)

class _Rng:

    def __init__(self, key):
        self._k = key

    def _next(self):
        self._k, sub = jax.random.split(self._k)
        return sub

    def normal(self, shape):
        return jax.random.normal(self._next(), shape, dtype=jnp.bfloat16)

    def randint(self, lo, hi, shape):
        return jax.random.randint(self._next(), shape, lo, hi, dtype=jnp.int32)

    def uniform(self, shape, lo=0.0, hi=1.0):
        return jax.random.uniform(self._next(), shape, jnp.bfloat16, lo, hi)

    def permutation(self, n):
        return jax.random.permutation(self._next(), n)
kernel_name = 'adaLN_cond__linear_kernel_hedgehog__geglu_ffn__prompt'

def setup_inputs():
    _rng = _Rng(jax.random.key(int.from_bytes(__import__("os").urandom(4), "little")))
    _w = lambda a: (lambda t: t.astype(jnp.bfloat16) if jnp.issubdtype(t.dtype, jnp.floating) else t)(jnp.asarray(a))

    def _A_setup():
        B, S, D, H = (1, 2048, 512, 32)
        Dh = D // H
        return {'x': _w((lambda *s: _rng.normal(s) * 0.05)(B, S, D)), 'wqkv': _w((lambda *s: _rng.normal(s) * 0.4)(D, 3 * D)), 'w_phi': _w((lambda *s: _rng.normal(s) * 0.4)(H, Dh, Dh) * Dh ** (-0.5)), 'wo': _w((lambda *s: _rng.normal(s) * 0.05)(D, D))}
    _A_in = _A_setup()

    def _B_setup():
        B, S, D, F = (1, 2048, 512, 1792)
        return {'x': _w((lambda *s: _rng.normal(s) * 0.05)(B, S, D)), 'w_gate': _w((lambda *s: _rng.normal(s) * 0.05)(D, F)), 'w_up': _w((lambda *s: _rng.normal(s) * 0.05)(D, F)), 'w_down': _w((lambda *s: _rng.normal(s) * 0.05)(F, D))}
    _B_in = _B_setup()
    return {'A_x': _A_in['x'], 'A_wqkv': _A_in['wqkv'], 'A_w_phi': _A_in['w_phi'], 'A_wo': _A_in['wo'], 'B_x': _B_in['x'], 'B_w_gate': _B_in['w_gate'], 'B_w_up': _B_in['w_up'], 'B_w_down': _B_in['w_down'], 'c': _w((lambda *s: _rng.normal(s) * 0.05)(1, 512) * 8.0), 'w_mod': _w((lambda *s: _rng.normal(s) * 0.05)(512, 6 * 512) * 512 ** (-0.5) * 8.0)}

def reference(A_x, A_wqkv, A_w_phi, A_wo, B_x, B_w_gate, B_w_up, B_w_down, c, w_mod):

    def _A_ref(x, wqkv, w_phi, wo):
        B, S, D = x.shape
        H = 32
        Dh = D // H
        qkv = (lambda x, *d: x.transpose(*d))((x @ wqkv).reshape(B, S, 3, H, Dh), 2, 0, 3, 1, 4)
        q, k, v = (qkv[0], qkv[1], qkv[2])
        pq = jnp.einsum('bhsd,hdf->bhsf', q, w_phi)
        pk = jnp.einsum('bhsd,hdf->bhsf', k, w_phi)
        phi_q = jnp.concatenate([_softmax(pq, axis=-1), _softmax(-pq, axis=-1)], axis=-1)
        phi_k = jnp.concatenate([_softmax(pk, axis=-1), _softmax(-pk, axis=-1)], axis=-1)
        kv = jnp.einsum('bhsf,bhsd->bhfd', phi_k, v)
        z = jnp.einsum('bhsf->bhf', phi_k)
        num = jnp.einsum('bhqf,bhfd->bhqd', phi_q, kv)
        den = jnp.einsum('bhqf,bhf->bhq', phi_q, z)[..., None] + 1e-06
        o = num / den
        return (lambda x, *d: x.transpose(*d))(o, 0, 2, 1, 3).reshape(B, S, D) @ wo

    def _B_ref(x, w_gate, w_up, w_down):
        return _gelu(x @ w_gate) * (x @ w_up) @ w_down
    x = A_x
    mod = (_silu(c) @ w_mod).reshape(c.shape[0], 6, 1, -1)
    sa, ca, ga, sb, cb, gb = (mod[:, 0].copy(), mod[:, 1].copy(), mod[:, 2].copy(), mod[:, 3].copy(), mod[:, 4].copy(), mod[:, 5].copy())
    h = _layernorm(x, axis=-1) * (1 + ca) + sa
    x = x + ga * _A_ref(h, A_wqkv, A_w_phi, A_wo)
    h = _layernorm(x, axis=-1) * (1 + cb) + sb
    x = x + gb * _B_ref(h, B_w_gate, B_w_up, B_w_down)
    return x
```

```python
import functools
import math
import jax
import jax.numpy as jnp
from jax import lax
import jax.experimental.pallas as pl
import jax.experimental.pallas.tpu as pltpu

S, D, H, DH, F = 2048, 512, 32, 16, 1792
T1 = 256
T2 = 256
FC = 256
U = 128
NG = 8
EPS_LN = 1e-5
EPS_DEN = 1e-6
LOG2E = math.log2(math.e)
BF = jnp.bfloat16
F32 = jnp.float32

NT = (((1,), (1,)), ((), ()))
TN = (((0,), (0,)), ((), ()))


def _dot(a, b):
    return jnp.dot(a, b, preferred_element_type=F32)


def _dg(a, b, dims):
    return lax.dot_general(a, b, dims, preferred_element_type=F32)


def _ln(x):
    m = jnp.mean(x, axis=-1, keepdims=True)
    xc = x - m
    v = jnp.mean(xc * xc, axis=-1, keepdims=True)
    return xc * lax.rsqrt(v + EPS_LN)


def _gelu(x):
    return jax.nn.gelu(x, approximate=True)


def _feat(p):
    T = p.shape[-1]
    p = p.reshape(8, 8, T)
    mx = jnp.max(p, axis=0)
    mx = jnp.maximum(mx, pltpu.roll(mx, 4, 0))
    mn = jnp.min(p, axis=0)
    mn = jnp.minimum(mn, pltpu.roll(mn, 4, 0))
    ep = jnp.exp2(p - mx[None])
    en = jnp.exp2(mn[None] - p)
    sp = jnp.sum(ep, axis=0)
    sp = sp + pltpu.roll(sp, 4, 0)
    sn = jnp.sum(en, axis=0)
    sn = sn + pltpu.roll(sn, 4, 0)
    e2 = jnp.concatenate([ep, en], axis=0).reshape(128, T)
    r2 = jnp.concatenate([jnp.broadcast_to((1.0 / sp)[None], (8, 8, T)),
                          jnp.broadcast_to((1.0 / sn)[None], (8, 8, T))], axis=0).reshape(128, T)
    return e2 * r2


def kernel(x_hbm, wqkv_hbm, wphi_hbm, wo_hbm, wg_hbm, wu_hbm, wd_hbm, c_hbm, wmod_hbm,
           out_hbm,
           x_v, wqkv_v, wphi_v, wo_v, wg_v, wu_v, wd_v, c_v, wmod_v,
           out_v, h_v, wt_v, kv_v, kvt_v, sems, osems):
    n1 = S // T1
    n2 = S // T2
    NU = S // U
    UPT = T1 // U

    def cp(src, dst, i):
        return pltpu.make_async_copy(src, dst, sems.at[i])

    c_c = cp(c_hbm, c_v, 0)
    c_m1a = cp(wmod_hbm.at[0:D // 2, 0:2 * D], wmod_v.at[0:D // 2, 0:2 * D], 1)
    c_m1b = cp(wmod_hbm.at[D // 2:D, 0:2 * D], wmod_v.at[D // 2:D, 0:2 * D], 16)
    c_phi = cp(wphi_hbm, wphi_v, 2)
    c_wq = cp(wqkv_hbm.at[:, 0:D], wqkv_v.at[:, 0:D], 3)
    c_m2 = cp(wmod_hbm.at[:, 2 * D:6 * D], wmod_v.at[:, 2 * D:6 * D], 4)
    c_wo = cp(wo_hbm, wo_v, 5)
    c_wg = cp(wg_hbm, wg_v, 6)
    c_wu = cp(wu_hbm, wu_v, 7)
    c_wd = cp(wd_hbm, wd_v, 8)
    c_wv = cp(wqkv_hbm.at[:, 2 * D:3 * D], wqkv_v.at[:, 2 * D:3 * D], 9)
    c_wk = cp(wqkv_hbm.at[:, D:2 * D], wqkv_v.at[:, D:2 * D], 10)
    XCH = [(0, 128), (128, 128), (256, 256), (512, 768), (1280, 768)]
    c_x = [cp(x_hbm.at[pl.ds(a, n)], x_v.at[pl.ds(a, n)], 11 + i) for i, (a, n) in enumerate(XCH)]
    xstart = {a // U: i for i, (a, n) in enumerate(XCH)}

    c_x[0].start(); c_phi.start(); c_wk.start(); c_c.start(); c_m1a.start(); c_m1b.start()

    c_phi.wait()
    p2 = wphi_v[...].reshape(DH * DH, H)
    r = lax.broadcasted_iota(jnp.int32, (H, D), 0)
    cc = lax.broadcasted_iota(jnp.int32, (H, D), 1)
    C = jnp.where(r == cc // DH, 1.0, 0.0).astype(BF)
    am = _dot(p2, C)
    r = lax.broadcasted_iota(jnp.int32, (DH * DH, D), 0)
    cc = lax.broadcasted_iota(jnp.int32, (DH * DH, D), 1)
    am = jnp.where(r // DH == cc % DH, am, 0.0).astype(BF)
    r = lax.broadcasted_iota(jnp.int32, (128, DH * DH), 0)
    cc = lax.broadcasted_iota(jnp.int32, (128, DH * DH), 1)
    E2 = jnp.where((r % 64) // 4 == cc % DH, 1.0, 0.0).astype(BF)
    mt = _dot(E2, am)
    r2 = lax.broadcasted_iota(jnp.int32, (128, D), 0)
    c2 = lax.broadcasted_iota(jnp.int32, (128, D), 1)
    mt = jnp.where((r2 // 64) * 4 + r2 % 4 == (c2 // DH) % 8, mt, 0.0).astype(BF)
    r = lax.broadcasted_iota(jnp.int32, (128, 128), 0)
    cc = lax.broadcasted_iota(jnp.int32, (128, 128), 1)
    eye = jnp.where(r == cc, 1.0, 0.0).astype(BF)

    c_x[0].wait()
    xn0 = _ln(x_v[pl.ds(0, U), :].astype(F32))
    c_wk.wait()

    def fold(col0, row0):
        for b in range(4):
            mb = mt[:, 128 * b:128 * (b + 1)]
            w = _dg(mb, wqkv_v[:, col0 + 128 * b:col0 + 128 * (b + 1)], NT)
            wt_v[row0 + 128 * b:row0 + 128 * (b + 1), :] = (w * LOG2E).astype(BF)

    fold(D, D)
    kv_v[...] = jnp.zeros(kv_v.shape, F32)

    c_c.wait(); c_m1a.wait()
    c_x[1].start(); c_wv.start(); c_x[2].start()
    cf = c_v[...].astype(F32)
    ca_act = (cf * jax.nn.sigmoid(cf)).astype(BF)
    c8 = jnp.broadcast_to(ca_act, (8, D))
    m1 = _dot(c8[:, 0:D // 2], wmod_v[0:D // 2, 0:2 * D])
    c_m1b.wait()
    m1 = m1 + _dot(c8[:, D // 2:D], wmod_v[D // 2:D, 0:2 * D])
    sa = m1[0:1, 0:D]
    ca1 = 1.0 + m1[0:1, D:2 * D]

    def ln1(u):
        xt = x_v[pl.ds(u * U, U), :].astype(F32)
        h = (_ln(xt) * ca1 + sa).astype(BF)
        h_v[pl.ds(u * U, U), :] = h
        return h

    def k_mm(h, b):
        return _dg(wt_v[D + 128 * b:D + 128 * (b + 1), :], h, NT)

    def v_mm(h, b):
        return _dg(wt_v[2 * D + 128 * b:2 * D + 128 * (b + 1), :], h, NT).astype(BF)

    ones16 = jnp.ones((16, U), BF)

    def kv_acc(pk, vt, g):
        o = 64 * (g % 2)
        ph = _feat(pk[g // 2][o:o + 64, :]).astype(BF)
        lhs = jnp.concatenate([vt[g // 2][o:o + 64, :], ones16], axis=0)
        kv_v[g] += _dg(lhs, ph, NT)

    h = (xn0 * ca1 + sa).astype(BF)
    h_v[pl.ds(0, U), :] = h
    pk = [k_mm(h, b) for b in range(4)]
    c_x[1].wait()
    hn = ln1(1)
    pk1 = [k_mm(hn, b) for b in range(4)]
    c_wv.wait(); c_x[2].wait()
    c_x[3].start(); c_x[4].start()
    c_wq.start()
    for b in range(4):
        wt_v[2 * D + 128 * b:2 * D + 128 * (b + 1), :] = _dg(
            eye, wqkv_v[:, 2 * D + 128 * b:2 * D + 128 * (b + 1)], NT).astype(BF)
    vt = [v_mm(h, b) for b in range(4)]
    for u in range(NU):
        if u + 2 < NU and (u + 2) in xstart and xstart[u + 2] >= 3:
            c_x[xstart[u + 2]].wait()
        if u == 2:
            c_wo.start(); c_m2.start(); c_wg.start(); c_wu.start(); c_wd.start()
        if u == 8:
            c_wq.wait(); c_m2.wait(); c_wo.wait()
            fold(0, 0)
        nx = u + 1 < NU
        pk_n = [None] * 4; vt_n = [None] * 4
        for b in range(4):
            if nx:
                pk_n[b] = pk1[b] if u == 0 else k_mm(hn, b)
            kv_acc(pk, vt, 2 * b)
            if nx:
                vt_n[b] = v_mm(hn, b)
            kv_acc(pk, vt, 2 * b + 1)
        pk, vt = pk_n, vt_n
        if u + 2 < NU:
            hn = ln1(u + 2)

    def a_pq(i):
        return _dg(wt_v[0:D, :], h_v[pl.ds(i * T2, T2), :], NT)

    pq = a_pq(0)
    ga = _dot(c8, wmod_v[:, 2 * D:3 * D])[0:1]

    r3 = lax.broadcasted_iota(jnp.int32, (80, 128), 0)
    c3 = lax.broadcasted_iota(jnp.int32, (80, 128), 1)
    msk = jnp.where(r3 < 64, r3 // DH, r3 % 4) == (c3 % 4)
    for g in range(NG):
        kvt_v[g] = jnp.where(msk, kv_v[g], 0.0).astype(BF)

    def out_copy(i, slot):
        return pltpu.make_async_copy(out_v.at[slot], out_hbm.at[pl.ds(i * T2, T2)], osems.at[slot])

    def a_head(pq, g):
        w = pq.shape[-1]
        ph = _feat(pq[64 * g:64 * (g + 1), :]).astype(BF)
        nd = _dot(kvt_v[g], ph)
        rd = 1.0 / (nd[64:72] + EPS_DEN)
        outs = [nd[16 * hl:16 * (hl + 1)] * jnp.broadcast_to(rd[hl:hl + 1], (16, w)) for hl in range(4)]
        return jnp.concatenate(outs, axis=0).astype(BF)

    def a_wo(ots, r0):
        ot = jnp.concatenate(ots, axis=0)
        attn = _dg(ot, wo_v[...], TN)
        return x_v[pl.ds(r0, ot.shape[-1]), :].astype(F32) + ga * attn

    def a_ln(x2):
        return (_ln(x2) * cb1 + sb).astype(BF)

    NC = F // FC

    def gu(h2, j):
        return (_dot(h2, wg_v[:, FC * j:FC * (j + 1)]), _dot(h2, wu_v[:, FC * j:FC * (j + 1)]))

    HW = T2 // 2
    otsa = [a_head(pq[:, 0:HW], g) for g in range(NG)]
    m3 = _dot(c8, wmod_v[:, 3 * D:5 * D])
    sb = m3[0:1, 0:D]
    cb1 = 1.0 + m3[0:1, D:2 * D]
    x2a = a_wo(otsa, 0)
    otsb = [a_head(pq[:, HW:T2], g) for g in range(NG)]
    gb = _dot(c8, wmod_v[:, 5 * D:6 * D])[0:1]
    x2b = a_wo(otsb, HW)
    h2a = a_ln(x2a)
    c_wg.wait(); c_wu.wait(); c_wd.wait()
    ga_, ua_ = gu(h2a, 0)
    h2b = a_ln(x2b)
    gb_, ub_ = gu(h2b, 0)
    x2 = jnp.concatenate([x2a, x2b], axis=0)
    h2 = jnp.concatenate([h2a, h2b], axis=0)
    g_ = jnp.concatenate([ga_, gb_], axis=0)
    u_ = jnp.concatenate([ua_, ub_], axis=0)
    for i in range(n2):
        slot = i % 2
        nxt = i + 1 < n2
        acc = None
        st = {}
        for j in range(NC):
            if j > 0:
                g_, u_ = gu(h2, j)
            if nxt:
                if j == 0:
                    st['pq'] = a_pq(i + 1)
                elif j in (1, 2):
                    for g in range(4 * (j - 1), 4 * j):
                        st['o', g] = a_head(st['pq'], g)
                elif j == 3:
                    st['x2'] = a_wo([st['o', g] for g in range(NG)], (i + 1) * T2)
                elif j == 4:
                    st['h2'] = a_ln(st['x2'])
            a = (_gelu(g_) * u_).astype(BF)
            d = _dot(a, wd_v[FC * j:FC * (j + 1), :])
            acc = d if acc is None else acc + d
        if nxt:
            g_, u_ = gu(st['h2'], 0)
        out_v[i] = (x2 + gb * acc).astype(BF)
        out_copy(i, i).start()
        if nxt:
            x2, h2 = st['x2'], st['h2']
    for i in range(n2):
        out_copy(i, i).wait()


@jax.jit
def pallas_adaLN_cond__linear_kernel_hedgehog__geglu_ffn__prompt_kernel(
    A_x, A_wqkv, A_w_phi, A_wo, B_x, B_w_gate, B_w_up, B_w_down, c, w_mod):
    x = A_x.reshape(S, D)
    wp = A_w_phi.transpose(1, 2, 0)
    n1 = S // T1
    any_spec = pl.BlockSpec(memory_space=pl.ANY)
    out = pl.pallas_call(
        kernel,
        out_shape=jax.ShapeDtypeStruct((S, D), BF),
        in_specs=[any_spec] * 9,
        out_specs=any_spec,
        scratch_shapes=[
            pltpu.VMEM((S, D), BF),
            pltpu.VMEM((D, 3 * D), BF),
            pltpu.VMEM((DH, DH, H), BF),
            pltpu.VMEM((D, D), BF),
            pltpu.VMEM((D, F), BF),
            pltpu.VMEM((D, F), BF),
            pltpu.VMEM((F, D), BF),
            pltpu.VMEM((1, D), BF),
            pltpu.VMEM((D, 6 * D), BF),
            pltpu.VMEM((S // T2, T2, D), BF),
            pltpu.VMEM((S, D), BF),
            pltpu.VMEM((3 * D, D), BF),
            pltpu.VMEM((NG, 80, 128), F32),
            pltpu.VMEM((NG, 80, 128), BF),
            pltpu.SemaphoreType.DMA((17,)),
            pltpu.SemaphoreType.DMA((S // T2,)),
        ],
        compiler_params=pltpu.CompilerParams(vmem_limit_bytes=100 * 1024 * 1024),
    )(x, A_wqkv, wp, A_wo, B_w_gate, B_w_up, B_w_down, c, w_mod)
    return out.reshape(1, S, D)
```

```python
import math
import jax
import jax.numpy as jnp
from jax import lax
import jax.experimental.pallas as pl
import jax.experimental.pallas.tpu as pltpu

S, D, H, DH, F = 2048, 512, 32, 16, 1792
T2 = 256
FC = 256
U = 128
NG = 8
NQ = 4
XCH = [(0, 128), (128, 128), (256, 256), (512, 768), (1280, 768)]
EPS_LN = 1e-5
EPS_DEN = 1e-6
LOG2E = math.log2(math.e)
BF = jnp.bfloat16
F32 = jnp.float32

NT = (((1,), (1,)), ((), ()))
TN = (((0,), (0,)), ((), ()))


def _dot(a, b):
    return jnp.dot(a, b, preferred_element_type=F32)


def _dg(a, b, dims):
    return lax.dot_general(a, b, dims, preferred_element_type=F32)


def _ln(x):
    m = jnp.mean(x, axis=-1, keepdims=True)
    xc = x - m
    v = jnp.mean(xc * xc, axis=-1, keepdims=True)
    return xc * lax.rsqrt(v + EPS_LN)


def _gelu(x):
    return jax.nn.gelu(x, approximate=True)


def _feat(p):
    T = p.shape[-1]
    p = p.reshape(8, 8, T)
    mx = jnp.max(p, axis=0)
    mx = jnp.maximum(mx, pltpu.roll(mx, 4, 0))
    mn = jnp.min(p, axis=0)
    mn = jnp.minimum(mn, pltpu.roll(mn, 4, 0))
    ep = jnp.exp2(p - mx[None])
    en = jnp.exp2(mn[None] - p)
    sp = jnp.sum(ep, axis=0)
    sp = sp + pltpu.roll(sp, 4, 0)
    sn = jnp.sum(en, axis=0)
    sn = sn + pltpu.roll(sn, 4, 0)
    e2 = jnp.concatenate([ep, en], axis=0).reshape(128, T)
    r2 = jnp.concatenate([jnp.broadcast_to((1.0 / sp)[None], (8, 8, T)),
                          jnp.broadcast_to((1.0 / sn)[None], (8, 8, T))], axis=0).reshape(128, T)
    return e2 * r2


def kernel(x_hbm, wqkv_hbm, wphi_hbm, wo_hbm, wg_hbm, wu_hbm, wd_hbm, c_hbm, wmod_hbm,
           out_hbm,
           x_v, wqkv_v, wphi_v, wo_v, wg_v, wu_v, wd_v, c_v, wmod_v,
           out_v, h_v, wt_v, kv_v, kvt_v, sems, osems):
    n2 = S // T2
    NU = S // U

    def cp(src, dst, i):
        return pltpu.make_async_copy(src, dst, sems.at[i])

    c_c = cp(c_hbm, c_v, 0)
    c_m1a = cp(wmod_hbm.at[0:D // 2, 0:2 * D], wmod_v.at[0:D // 2, 0:2 * D], 1)
    c_m1b = cp(wmod_hbm.at[D // 2:D, 0:2 * D], wmod_v.at[D // 2:D, 0:2 * D], 16)
    c_phi = cp(wphi_hbm, wphi_v, 2)
    c_wq = cp(wqkv_hbm.at[:, 0:D], wqkv_v.at[:, 0:D], 3)
    c_m2 = cp(wmod_hbm.at[:, 2 * D:6 * D], wmod_v.at[:, 2 * D:6 * D], 4)
    c_wo = cp(wo_hbm, wo_v, 5)
    c_wg = cp(wg_hbm, wg_v, 6)
    c_wu = cp(wu_hbm, wu_v, 7)
    c_wd = cp(wd_hbm, wd_v, 8)
    c_wv = cp(wqkv_hbm.at[:, 2 * D:3 * D], wqkv_v.at[:, 2 * D:3 * D], 9)
    c_wk = cp(wqkv_hbm.at[:, D:2 * D], wqkv_v.at[:, D:2 * D], 10)
    c_x = [cp(x_hbm.at[pl.ds(a, n)], x_v.at[pl.ds(a, n)], 11 + i) for i, (a, n) in enumerate(XCH)]
    xstart = {a // U: i for i, (a, n) in enumerate(XCH)}

    c_x[0].start(); c_phi.start(); c_wk.start(); c_c.start(); c_m1a.start(); c_m1b.start()

    c_phi.wait()
    p2 = wphi_v[...].reshape(DH * DH, H)
    r = lax.broadcasted_iota(jnp.int32, (H, D), 0)
    cc = lax.broadcasted_iota(jnp.int32, (H, D), 1)
    C = jnp.where(r == cc // DH, 1.0, 0.0).astype(BF)
    am = _dot(p2, C)
    r = lax.broadcasted_iota(jnp.int32, (DH * DH, D), 0)
    cc = lax.broadcasted_iota(jnp.int32, (DH * DH, D), 1)
    am = jnp.where(r // DH == cc % DH, am, 0.0).astype(BF)
    r = lax.broadcasted_iota(jnp.int32, (128, DH * DH), 0)
    cc = lax.broadcasted_iota(jnp.int32, (128, DH * DH), 1)
    E2 = jnp.where((r % 64) // 4 == cc % DH, 1.0, 0.0).astype(BF)
    mt = _dot(E2, am)
    r2 = lax.broadcasted_iota(jnp.int32, (128, D), 0)
    c2 = lax.broadcasted_iota(jnp.int32, (128, D), 1)
    mt = jnp.where((r2 // 64) * 4 + r2 % 4 == (c2 // DH) % 8, mt, 0.0).astype(BF)
    r = lax.broadcasted_iota(jnp.int32, (128, 128), 0)
    cc = lax.broadcasted_iota(jnp.int32, (128, 128), 1)
    eye = jnp.where(r == cc, 1.0, 0.0).astype(BF)

    c_x[0].wait()
    xn0 = _ln(x_v[pl.ds(0, U), :].astype(F32))
    c_wk.wait()

    def fold(col0, row0):
        for b in range(4):
            mb = mt[:, 128 * b:128 * (b + 1)]
            w = _dg(mb, wqkv_v[:, col0 + 128 * b:col0 + 128 * (b + 1)], NT)
            wt_v[row0 + 128 * b:row0 + 128 * (b + 1), :] = (w * LOG2E).astype(BF)

    fold(D, D)
    kv_v[...] = jnp.zeros(kv_v.shape, F32)

    c_c.wait(); c_m1a.wait()
    c_x[1].start(); c_wv.start(); c_x[2].start()
    cf = c_v[...].astype(F32)
    ca_act = (cf * jax.nn.sigmoid(cf)).astype(BF)
    c8 = jnp.broadcast_to(ca_act, (8, D))
    m1 = _dot(c8[:, 0:D // 2], wmod_v[0:D // 2, 0:2 * D])
    c_m1b.wait()
    m1 = m1 + _dot(c8[:, D // 2:D], wmod_v[D // 2:D, 0:2 * D])
    sa = m1[0:1, 0:D]
    ca1 = 1.0 + m1[0:1, D:2 * D]

    def ln1(u):
        xt = x_v[pl.ds(u * U, U), :].astype(F32)
        h = (_ln(xt) * ca1 + sa).astype(BF)
        h_v[pl.ds(u * U, U), :] = h
        return h

    def k_mm(h, b):
        return _dg(wt_v[D + 128 * b:D + 128 * (b + 1), :], h, NT)

    def v_mm(h, b):
        return _dg(wt_v[2 * D + 128 * b:2 * D + 128 * (b + 1), :], h, NT).astype(BF)

    ones16 = jnp.ones((16, U), BF)

    def kv_acc(pk, vt, g):
        o = 64 * (g % 2)
        ph = _feat(pk[g // 2][o:o + 64, :]).astype(BF)
        lhs = jnp.concatenate([vt[g // 2][o:o + 64, :], ones16], axis=0)
        kv_v[g] += _dg(lhs, ph, NT)

    h = (xn0 * ca1 + sa).astype(BF)
    h_v[pl.ds(0, U), :] = h
    pk = [k_mm(h, b) for b in range(4)]
    c_x[1].wait()
    hn = ln1(1)
    pk1 = [k_mm(hn, b) for b in range(4)]
    c_wv.wait(); c_x[2].wait()
    c_x[3].start(); c_x[4].start()
    c_wq.start()
    for b in range(4):
        wt_v[2 * D + 128 * b:2 * D + 128 * (b + 1), :] = _dg(
            eye, wqkv_v[:, 2 * D + 128 * b:2 * D + 128 * (b + 1)], NT).astype(BF)
    vt = [v_mm(h, b) for b in range(4)]
    for u in range(NU):
        if u + 2 < NU and (u + 2) in xstart and xstart[u + 2] >= 3:
            c_x[xstart[u + 2]].wait()
        if u == 2:
            c_wo.start(); c_m2.start(); c_wg.start(); c_wu.start(); c_wd.start()
        if u == 8:
            c_wq.wait(); c_m2.wait(); c_wo.wait()
            fold(0, 0)
        nx = u + 1 < NU
        pk_n = [None] * 4; vt_n = [None] * 4
        for b in range(4):
            if nx:
                pk_n[b] = pk1[b] if u == 0 else k_mm(hn, b)
            kv_acc(pk, vt, 2 * b)
            if nx:
                vt_n[b] = v_mm(hn, b)
            kv_acc(pk, vt, 2 * b + 1)
        pk, vt = pk_n, vt_n
        if u + 2 < NU:
            hn = ln1(u + 2)

    def a_pq(i):
        return _dg(wt_v[0:D, :], h_v[pl.ds(i * T2, T2), :], NT)

    pq = a_pq(0)
    ga = _dot(c8, wmod_v[:, 2 * D:3 * D])[0:1]

    r3 = lax.broadcasted_iota(jnp.int32, (80, 128), 0)
    c3 = lax.broadcasted_iota(jnp.int32, (80, 128), 1)
    msk = jnp.where(r3 < 64, r3 // DH, r3 % 4) == (c3 % 4)
    for g in range(NG):
        kvt_v[g] = jnp.where(msk, kv_v[g], 0.0).astype(BF)

    def out_copy(i):
        return pltpu.make_async_copy(out_v.at[i], out_hbm.at[pl.ds(i * T2, T2)], osems.at[i])

    QR = T2 // NQ

    def tail_copy(q):
        return pltpu.make_async_copy(out_v.at[n2 - 1, pl.ds(q * QR, QR)],
                                     out_hbm.at[pl.ds((n2 - 1) * T2 + q * QR, QR)], osems.at[n2 - 1 + q])

    def a_head(pq, g):
        w = pq.shape[-1]
        ph = _feat(pq[64 * g:64 * (g + 1), :]).astype(BF)
        nd = _dot(kvt_v[g], ph)
        rd = 1.0 / (nd[64:72] + EPS_DEN)
        outs = [nd[16 * hl:16 * (hl + 1)] * jnp.broadcast_to(rd[hl:hl + 1], (16, w)) for hl in range(4)]
        return jnp.concatenate(outs, axis=0).astype(BF)

    def a_wo(ots, r0):
        ot = jnp.concatenate(ots, axis=0)
        attn = _dg(ot, wo_v[...], TN)
        return x_v[pl.ds(r0, ot.shape[-1]), :].astype(F32) + ga * attn

    def a_ln(x2):
        return (_ln(x2) * cb1 + sb).astype(BF)

    NC = F // FC

    def gu(h2, j):
        return (_dot(h2, wg_v[:, FC * j:FC * (j + 1)]), _dot(h2, wu_v[:, FC * j:FC * (j + 1)]))

    HW = T2 // 2
    otsa = [a_head(pq[:, 0:HW], g) for g in range(NG)]
    m3 = _dot(c8, wmod_v[:, 3 * D:5 * D])
    sb = m3[0:1, 0:D]
    cb1 = 1.0 + m3[0:1, D:2 * D]
    x2a = a_wo(otsa, 0)
    otsb = [a_head(pq[:, HW:T2], g) for g in range(NG)]
    gb = _dot(c8, wmod_v[:, 5 * D:6 * D])[0:1]
    x2b = a_wo(otsb, HW)
    h2a = a_ln(x2a)
    c_wg.wait(); c_wu.wait(); c_wd.wait()
    ga_, ua_ = gu(h2a, 0)
    h2b = a_ln(x2b)
    gb_, ub_ = gu(h2b, 0)
    x2 = jnp.concatenate([x2a, x2b], axis=0)
    h2 = jnp.concatenate([h2a, h2b], axis=0)
    g_ = jnp.concatenate([ga_, gb_], axis=0)
    u_ = jnp.concatenate([ua_, ub_], axis=0)
    for i in range(n2):
        nxt = i + 1 < n2
        acc = None
        st = {}
        for j in range(NC):
            if j > 0:
                g_, u_ = gu(h2, j)
            if nxt:
                if j == 0:
                    st['pq'] = a_pq(i + 1)
                elif j in (1, 2):
                    for g in range(4 * (j - 1), 4 * j):
                        st['o', g] = a_head(st['pq'], g)
                elif j == 3:
                    st['x2'] = a_wo([st['o', g] for g in range(NG)], (i + 1) * T2)
                elif j == 4:
                    st['h2'] = a_ln(st['x2'])
            a = (_gelu(g_) * u_).astype(BF)
            if nxt or j + 1 < NC:
                d = _dot(a, wd_v[FC * j:FC * (j + 1), :])
                acc = d if acc is None else acc + d
        if nxt:
            g_, u_ = gu(st['h2'], 0)
            out_v[i] = (x2 + gb * acc).astype(BF)
            out_copy(i).start()
            x2, h2 = st['x2'], st['h2']
        else:
            for q in range(NQ):
                rs = slice(q * QR, (q + 1) * QR)
                dq = _dot(a[rs], wd_v[FC * (NC - 1):FC * NC, :])
                out_v[i, rs, :] = (x2[rs] + gb * (acc[rs] + dq)).astype(BF)
                tail_copy(q).start()
    for i in range(n2 - 1):
        out_copy(i).wait()
    for q in range(NQ):
        tail_copy(q).wait()


@jax.jit
def pallas_adaLN_cond__linear_kernel_hedgehog__geglu_ffn__prompt_kernel(
    A_x, A_wqkv, A_w_phi, A_wo, B_x, B_w_gate, B_w_up, B_w_down, c, w_mod):
    x = A_x.reshape(S, D)
    wp = A_w_phi.transpose(1, 2, 0)
    any_spec = pl.BlockSpec(memory_space=pl.ANY)
    out = pl.pallas_call(
        kernel,
        out_shape=jax.ShapeDtypeStruct((S, D), BF),
        in_specs=[any_spec] * 9,
        out_specs=any_spec,
        scratch_shapes=[
            pltpu.VMEM((S, D), BF),
            pltpu.VMEM((D, 3 * D), BF),
            pltpu.VMEM((DH, DH, H), BF),
            pltpu.VMEM((D, D), BF),
            pltpu.VMEM((D, F), BF),
            pltpu.VMEM((D, F), BF),
            pltpu.VMEM((F, D), BF),
            pltpu.VMEM((1, D), BF),
            pltpu.VMEM((D, 6 * D), BF),
            pltpu.VMEM((S // T2, T2, D), BF),
            pltpu.VMEM((S, D), BF),
            pltpu.VMEM((3 * D, D), BF),
            pltpu.VMEM((NG, 80, 128), F32),
            pltpu.VMEM((NG, 80, 128), BF),
            pltpu.SemaphoreType.DMA((17,)),
            pltpu.SemaphoreType.DMA((S // T2 + NQ - 1,)),
        ],
        compiler_params=pltpu.CompilerParams(vmem_limit_bytes=100 * 1024 * 1024),
    )(x, A_wqkv, wp, A_wo, B_w_gate, B_w_up, B_w_down, c, w_mod)
    return out.reshape(1, S, D)
```

```python
import math
import jax
import jax.numpy as jnp
from jax import lax
import jax.experimental.pallas as pl
import jax.experimental.pallas.tpu as pltpu

S, D, H, DH, F = 2048, 512, 32, 16, 1792
T2 = 256
FC = 256
U = 128
NG = 8
NQ = 4
XCH = [(0, 128), (128, 128), (256, 256), (512, 768), (1280, 768)]
EPS_LN = 1e-5
EPS_DEN = 1e-6
LOG2E = math.log2(math.e)
BF = jnp.bfloat16
F32 = jnp.float32

NT = (((1,), (1,)), ((), ()))
TN = (((0,), (0,)), ((), ()))


def _dot(a, b):
    return jnp.dot(a, b, preferred_element_type=F32)


def _dg(a, b, dims):
    return lax.dot_general(a, b, dims, preferred_element_type=F32)


def _ln(x):
    m = jnp.mean(x, axis=-1, keepdims=True)
    xc = x - m
    v = jnp.mean(xc * xc, axis=-1, keepdims=True)
    return xc * lax.rsqrt(v + EPS_LN)


def _gelu(x):
    return jax.nn.gelu(x, approximate=True)


def _feat(p):
    T = p.shape[-1]
    p = p.reshape(8, 8, T)
    mx = jnp.max(p, axis=0)
    mx = jnp.maximum(mx, pltpu.roll(mx, 4, 0))
    mn = jnp.min(p, axis=0)
    mn = jnp.minimum(mn, pltpu.roll(mn, 4, 0))
    ep = jnp.exp2(p - mx[None])
    en = jnp.exp2(mn[None] - p)
    sp = jnp.sum(ep, axis=0)
    sp = sp + pltpu.roll(sp, 4, 0)
    sn = jnp.sum(en, axis=0)
    sn = sn + pltpu.roll(sn, 4, 0)
    e2 = jnp.concatenate([ep, en], axis=0).reshape(128, T)
    r2 = jnp.concatenate([jnp.broadcast_to((1.0 / sp)[None], (8, 8, T)),
                          jnp.broadcast_to((1.0 / sn)[None], (8, 8, T))], axis=0).reshape(128, T)
    return e2 * r2


def kernel(x_hbm, wqkv_hbm, wphi_hbm, wo_hbm, wg_hbm, wu_hbm, wd_hbm, c_hbm, wmod_hbm,
           out_hbm,
           x_v, wqkv_v, wphi_v, wo_v, wg_v, wu_v, wd_v, c_v, wmod_v,
           out_v, h_v, wt_v, kv_v, kvt_v, pk_v, sems, osems):
    n2 = S // T2
    NU = S // U

    def cp(src, dst, i):
        return pltpu.make_async_copy(src, dst, sems.at[i])

    c_c = cp(c_hbm, c_v, 0)
    c_ca = cp(wmod_hbm.at[:, D:2 * D], wmod_v.at[:, D:2 * D], 1)
    c_sa = cp(wmod_hbm.at[:, 0:D], wmod_v.at[:, 0:D], 16)
    c_phi = cp(wphi_hbm, wphi_v, 2)
    c_wq = cp(wqkv_hbm.at[:, 0:D], wqkv_v.at[:, 0:D], 3)
    c_m2 = cp(wmod_hbm.at[:, 2 * D:6 * D], wmod_v.at[:, 2 * D:6 * D], 4)
    c_wo = cp(wo_hbm, wo_v, 5)
    c_wg = cp(wg_hbm, wg_v, 6)
    c_wu = cp(wu_hbm, wu_v, 7)
    c_wd = cp(wd_hbm, wd_v, 8)
    c_wv = cp(wqkv_hbm.at[:, 2 * D:3 * D], wqkv_v.at[:, 2 * D:3 * D], 9)
    c_wk = cp(wqkv_hbm.at[:, D:2 * D], wqkv_v.at[:, D:2 * D], 10)
    c_x = [cp(x_hbm.at[pl.ds(a, n)], x_v.at[pl.ds(a, n)], 11 + i) for i, (a, n) in enumerate(XCH)]

    c_x[0].start(); c_phi.start(); c_wk.start(); c_c.start(); c_ca.start()
    c_x[1].start(); c_x[2].start(); c_sa.start(); c_wv.start(); c_x[3].start()

    c_phi.wait()
    p2 = wphi_v[...].reshape(DH * DH, H)
    r = lax.broadcasted_iota(jnp.int32, (H, D), 0)
    cc = lax.broadcasted_iota(jnp.int32, (H, D), 1)
    C = jnp.where(r == cc // DH, 1.0, 0.0).astype(BF)
    am = _dot(p2, C)
    r = lax.broadcasted_iota(jnp.int32, (DH * DH, D), 0)
    cc = lax.broadcasted_iota(jnp.int32, (DH * DH, D), 1)
    am = jnp.where(r // DH == cc % DH, am, 0.0).astype(BF)
    r = lax.broadcasted_iota(jnp.int32, (128, DH * DH), 0)
    cc = lax.broadcasted_iota(jnp.int32, (128, DH * DH), 1)
    E2 = jnp.where((r % 64) // 4 == cc % DH, 1.0, 0.0).astype(BF)
    mt = _dot(E2, am)
    r2 = lax.broadcasted_iota(jnp.int32, (128, D), 0)
    c2 = lax.broadcasted_iota(jnp.int32, (128, D), 1)
    mt = jnp.where((r2 // 64) * 4 + r2 % 4 == (c2 // DH) % 8, mt, 0.0).astype(BF)
    r = lax.broadcasted_iota(jnp.int32, (128, 128), 0)
    cc = lax.broadcasted_iota(jnp.int32, (128, 128), 1)
    eye = jnp.where(r == cc, 1.0, 0.0).astype(BF)

    c_x[0].wait()
    xn0 = _ln(x_v[pl.ds(0, U), :].astype(F32))
    c_wk.wait()

    def fold(col0, row0):
        for b in range(4):
            mb = mt[:, 128 * b:128 * (b + 1)]
            w = _dg(mb, wqkv_v[:, col0 + 128 * b:col0 + 128 * (b + 1)], NT)
            wt_v[row0 + 128 * b:row0 + 128 * (b + 1), :] = (w * LOG2E).astype(BF)

    fold(D, D)
    kv_v[...] = jnp.zeros(kv_v.shape, F32)

    c_c.wait(); c_ca.wait()
    cf = c_v[...].astype(F32)
    ca_act = (cf * jax.nn.sigmoid(cf)).astype(BF)
    c8 = jnp.broadcast_to(ca_act, (8, D))
    ca1 = 1.0 + _dot(c8, wmod_v[:, D:2 * D])[0:1]

    def ln1(u):
        xt = x_v[pl.ds(u * U, U), :].astype(F32)
        h = (_ln(xt) * ca1 + sa).astype(BF)
        h_v[pl.ds(u * U, U), :] = h
        return h

    def k_mm(h, b):
        return _dg(wt_v[D + 128 * b:D + 128 * (b + 1), :], h, NT)

    def v_mm(h, b):
        return _dg(wt_v[2 * D + 128 * b:2 * D + 128 * (b + 1), :], h, NT).astype(BF)

    ones16 = jnp.ones((16, U), BF)

    def kv_acc(pk, vt, g):
        o = 64 * (g % 2)
        ph = _feat(pk[g // 2][o:o + 64, :]).astype(BF)
        lhs = jnp.concatenate([vt[g // 2][o:o + 64, :], ones16], axis=0)
        kv_v[g] += _dg(lhs, ph, NT)

    NP = 2
    xs = {0: xn0 * ca1}
    x0b = xs[0].astype(BF)
    c_x[1].wait()
    xs[1] = _ln(x_v[pl.ds(U, U), :].astype(F32)) * ca1
    x1b = xs[1].astype(BF)
    for b in range(4):
        pk_v[0, b] = k_mm(x0b, b)
    c_x[2].wait()
    xs[2] = _ln(x_v[pl.ds(2 * U, U), :].astype(F32)) * ca1
    for b in range(4):
        pk_v[1, b] = k_mm(x1b, b)
    c_sa.wait()
    sa = _dot(c8, wmod_v[:, 0:D])[0:1]
    sa_rows = jnp.broadcast_to(sa.astype(BF), (U, D))
    hh = {}
    for u in range(3):
        hh[u] = (xs[u] + sa).astype(BF)
        h_v[pl.ds(u * U, U), :] = hh[u]
    pk = {u: [None] * 4 for u in range(NP)}
    for b in range(4):
        bias = k_mm(sa_rows, b)
        for u in range(NP):
            pk[u][b] = pk_v[u, b] + bias
    pk[2] = [k_mm(hh[2], b) for b in range(4)]
    c_wv.wait()
    c_x[4].start()
    c_wq.start()
    for b in range(4):
        wt_v[2 * D + 128 * b:2 * D + 128 * (b + 1), :] = _dg(
            eye, wqkv_v[:, 2 * D + 128 * b:2 * D + 128 * (b + 1)], NT).astype(BF)
    vt = {0: [v_mm(hh[0], b) for b in range(4)]}
    hh[3] = ln1(3)

    for u in range(NU):
        if u == 1:
            c_x[3].wait()
            c_wo.start(); c_m2.start(); c_wg.start(); c_wu.start(); c_wd.start()
        if u == 7:
            c_x[4].wait(); c_wq.wait()
            fold(0, 0)
        if u == 12:
            c_m2.wait(); c_wo.wait()
        uk, ul = u + 2, u + 3
        do_k = 3 <= uk < NU
        if do_k:
            pk[uk] = [None] * 4
        if u + 1 < NU:
            vt[u + 1] = [None] * 4
        for b in range(4):
            kv_acc(pk[u], vt[u], 2 * b)
            if do_k:
                pk[uk][b] = k_mm(hh[uk], b)
            kv_acc(pk[u], vt[u], 2 * b + 1)
            if u + 1 < NU:
                vt[u + 1][b] = v_mm(hh[u + 1], b)
        if 3 < ul < NU:
            hh[ul] = ln1(ul)

    def a_pq(i):
        return _dg(wt_v[0:D, :], h_v[pl.ds(i * T2, T2), :], NT)

    pq = a_pq(0)
    ga = _dot(c8, wmod_v[:, 2 * D:3 * D])[0:1]

    r3 = lax.broadcasted_iota(jnp.int32, (80, 128), 0)
    c3 = lax.broadcasted_iota(jnp.int32, (80, 128), 1)
    msk = jnp.where(r3 < 64, r3 // DH, r3 % 4) == (c3 % 4)
    for g in range(NG):
        kvt_v[g] = jnp.where(msk, kv_v[g], 0.0).astype(BF)

    def out_copy(i):
        return pltpu.make_async_copy(out_v.at[i], out_hbm.at[pl.ds(i * T2, T2)], osems.at[i])

    QR = T2 // NQ

    def tail_copy(q):
        return pltpu.make_async_copy(out_v.at[n2 - 1, pl.ds(q * QR, QR)],
                                     out_hbm.at[pl.ds((n2 - 1) * T2 + q * QR, QR)], osems.at[n2 - 1 + q])

    def a_head(pq, g):
        w = pq.shape[-1]
        ph = _feat(pq[64 * g:64 * (g + 1), :]).astype(BF)
        nd = _dot(kvt_v[g], ph)
        rd = 1.0 / (nd[64:72] + EPS_DEN)
        outs = [nd[16 * hl:16 * (hl + 1)] * jnp.broadcast_to(rd[hl:hl + 1], (16, w)) for hl in range(4)]
        return jnp.concatenate(outs, axis=0).astype(BF)

    def a_wo(ots, r0):
        ot = jnp.concatenate(ots, axis=0)
        attn = _dg(ot, wo_v[...], TN)
        return x_v[pl.ds(r0, ot.shape[-1]), :].astype(F32) + ga * attn

    def a_ln(x2):
        return (_ln(x2) * cb1 + sb).astype(BF)

    NC = F // FC

    def gu(h2, j):
        return (_dot(h2, wg_v[:, FC * j:FC * (j + 1)]), _dot(h2, wu_v[:, FC * j:FC * (j + 1)]))

    HW = T2 // 2
    otsa = [a_head(pq[:, 0:HW], g) for g in range(NG)]
    m3 = _dot(c8, wmod_v[:, 3 * D:5 * D])
    sb = m3[0:1, 0:D]
    cb1 = 1.0 + m3[0:1, D:2 * D]
    x2a = a_wo(otsa, 0)
    otsb = [a_head(pq[:, HW:T2], g) for g in range(NG)]
    gb = _dot(c8, wmod_v[:, 5 * D:6 * D])[0:1]
    x2b = a_wo(otsb, HW)
    h2a = a_ln(x2a)
    c_wg.wait(); c_wu.wait(); c_wd.wait()
    ga_, ua_ = gu(h2a, 0)
    h2b = a_ln(x2b)
    gb_, ub_ = gu(h2b, 0)
    x2 = jnp.concatenate([x2a, x2b], axis=0)
    h2 = jnp.concatenate([h2a, h2b], axis=0)
    g_ = jnp.concatenate([ga_, gb_], axis=0)
    u_ = jnp.concatenate([ua_, ub_], axis=0)
    for i in range(n2):
        nxt = i + 1 < n2
        acc = None
        st = {}
        for j in range(NC):
            if j > 0:
                g_, u_ = gu(h2, j)
            if nxt:
                if j == 0:
                    st['pq'] = a_pq(i + 1)
                elif j in (1, 2):
                    for g in range(4 * (j - 1), 4 * j):
                        st['o', g] = a_head(st['pq'], g)
                elif j == 3:
                    st['x2'] = a_wo([st['o', g] for g in range(NG)], (i + 1) * T2)
                elif j == 4:
                    st['h2'] = a_ln(st['x2'])
            a = (_gelu(g_) * u_).astype(BF)
            if nxt or j + 1 < NC:
                d = _dot(a, wd_v[FC * j:FC * (j + 1), :])
                acc = d if acc is None else acc + d
        if nxt:
            g_, u_ = gu(st['h2'], 0)
            out_v[i] = (x2 + gb * acc).astype(BF)
            out_copy(i).start()
            x2, h2 = st['x2'], st['h2']
        else:
            for q in range(NQ):
                rs = slice(q * QR, (q + 1) * QR)
                dq = _dot(a[rs], wd_v[FC * (NC - 1):FC * NC, :])
                out_v[i, rs, :] = (x2[rs] + gb * (acc[rs] + dq)).astype(BF)
                tail_copy(q).start()
    for i in range(n2 - 1):
        out_copy(i).wait()
    for q in range(NQ):
        tail_copy(q).wait()


@jax.jit
def pallas_adaLN_cond__linear_kernel_hedgehog__geglu_ffn__prompt_kernel(
    A_x, A_wqkv, A_w_phi, A_wo, B_x, B_w_gate, B_w_up, B_w_down, c, w_mod):
    x = A_x.reshape(S, D)
    wp = A_w_phi.transpose(1, 2, 0)
    any_spec = pl.BlockSpec(memory_space=pl.ANY)
    out = pl.pallas_call(
        kernel,
        out_shape=jax.ShapeDtypeStruct((S, D), BF),
        in_specs=[any_spec] * 9,
        out_specs=any_spec,
        scratch_shapes=[
            pltpu.VMEM((S, D), BF),
            pltpu.VMEM((D, 3 * D), BF),
            pltpu.VMEM((DH, DH, H), BF),
            pltpu.VMEM((D, D), BF),
            pltpu.VMEM((D, F), BF),
            pltpu.VMEM((D, F), BF),
            pltpu.VMEM((F, D), BF),
            pltpu.VMEM((1, D), BF),
            pltpu.VMEM((D, 6 * D), BF),
            pltpu.VMEM((S // T2, T2, D), BF),
            pltpu.VMEM((S, D), BF),
            pltpu.VMEM((3 * D, D), BF),
            pltpu.VMEM((NG, 80, 128), F32),
            pltpu.VMEM((NG, 80, 128), BF),
            pltpu.VMEM((2, 4, 128, U), F32),
            pltpu.SemaphoreType.DMA((17,)),
            pltpu.SemaphoreType.DMA((S // T2 + NQ - 1,)),
        ],
        compiler_params=pltpu.CompilerParams(vmem_limit_bytes=100 * 1024 * 1024),
    )(x, A_wqkv, wp, A_wo, B_w_gate, B_w_up, B_w_down, c, w_mod)
    return out.reshape(1, S, D)
```
